```python
import os as _os
_os.environ.setdefault("JAX_PLATFORMS", "cpu")
import jax
import jax.numpy as jnp

def _softmax(x, axis=-1):
    return jax.nn.softmax(x, axis=axis)
def _gelu(x):
    return jax.nn.gelu(x, approximate=True)
def _silu(x):
    return jax.nn.silu(x)
def _sigmoid(x):
    return jax.nn.sigmoid(x)
def _layernorm(x, axis=-1, eps=1e-5):
    m = jnp.mean(x, axis=axis, keepdims=True)
    v = jnp.var(x, axis=axis, keepdims=True)
    return (x - m) / jnp.sqrt(v + eps)
def _scatter_add(tgt, idx, src, axis=0):
    return tgt.at[idx].add(src)
def _segment_sum(src, seg, n):
    return jax.ops.segment_sum(src, seg, n)
class _Rng:
    def __init__(self, key):
        self._k = key
    def _next(self):
        self._k, sub = jax.random.split(self._k)
        return sub
    def normal(self, shape):
        return jax.random.normal(self._next(), shape, dtype=jnp.bfloat16)
    def randint(self, lo, hi, shape):
        return jax.random.randint(self._next(), shape, lo, hi, dtype=jnp.int32)
    def uniform(self, shape, lo=0.0, hi=1.0):
        return jax.random.uniform(self._next(), shape, jnp.bfloat16, lo, hi)
    def permutation(self, n):
        return jax.random.permutation(self._next(), n)


kernel_name = 'concat_heads__gqa_block_cached__gqa_block_cached__near_ridge'

def setup_inputs():
    _rng = _Rng(jax.random.key(int.from_bytes(__import__("os").urandom(4), "little")))
    _w = (lambda a: (lambda t: t.astype(jnp.bfloat16) if jnp.issubdtype(t.dtype, jnp.floating) else t)(jnp.asarray(a)))
    def _A_setup():
        B, Sq, D = 8, 128, 576
        Hq, Hkv, Sk, Dh = 32, 16, 512, 128
        assert Hq % Hkv == 0, (Hq, Hkv)
        return {
            "x": _w((lambda *s: _rng.normal(s) * 0.8)(B, Sq, D)),
            "k_cache": _w((lambda *s: _rng.normal(s) * 0.8)(B, Hkv, Sk, Dh)),
            "v_cache": _w((lambda *s: _rng.normal(s) * 0.05)(B, Hkv, Sk, Dh)),
            "wq": _w((lambda *s: _rng.normal(s) * 0.8)(D, Hq * Dh) * (D ** -0.5)),
            "wo": _w((lambda *s: _rng.normal(s) * 0.05)(Hq * Dh, D) * ((Hq * Dh) ** -0.5)),
        }
    _A_in = _A_setup()

    def _B_setup():
        B, Sq, D = 8, 128, 576
        Hq, Hkv, Sk, Dh = 32, 16, 512, 128
        assert Hq % Hkv == 0, (Hq, Hkv)
        return {
            "x": _w((lambda *s: _rng.normal(s) * 0.8)(B, Sq, D)),
            "k_cache": _w((lambda *s: _rng.normal(s) * 0.8)(B, Hkv, Sk, Dh)),
            "v_cache": _w((lambda *s: _rng.normal(s) * 0.05)(B, Hkv, Sk, Dh)),
            "wq": _w((lambda *s: _rng.normal(s) * 0.8)(D, Hq * Dh) * (D ** -0.5)),
            "wo": _w((lambda *s: _rng.normal(s) * 0.05)(Hq * Dh, D) * ((Hq * Dh) ** -0.5)),
        }
    _B_in = _B_setup()

    return {
        "A_x": _A_in["x"],
        "A_k_cache": _A_in["k_cache"],
        "A_v_cache": _A_in["v_cache"],
        "A_wq": _A_in["wq"],
        "A_wo": _A_in["wo"],
        "B_x": _B_in["x"],
        "B_k_cache": _B_in["k_cache"],
        "B_v_cache": _B_in["v_cache"],
        "B_wq": _B_in["wq"],
        "B_wo": _B_in["wo"],
    }

def reference(A_x, A_k_cache, A_v_cache, A_wq, A_wo, B_x, B_k_cache, B_v_cache, B_wq, B_wo):
    def _A_ref(x, k_cache, v_cache, wq, wo):
        B, Sq, D = x.shape
        Hq, Dh = 32, 128
        Hkv = k_cache.shape[1]
        rep = Hq // Hkv
        q = (lambda x, *d: x.transpose(*d))((x @ wq).reshape(B, Sq, Hq, Dh), 0, 2, 1, 3)
        k = jnp.repeat(k_cache, rep, axis=1)
        v = jnp.repeat(v_cache, rep, axis=1)
        scores = jnp.einsum("bhqd,bhkd->bhqk", q, k) * (Dh ** -0.5)
        p = _softmax(scores, axis=-1)
        o = jnp.einsum("bhqk,bhkd->bhqd", p, v)
        return (lambda x, *d: x.transpose(*d))(o, 0, 2, 1, 3).reshape(B, Sq, Hq * Dh) @ wo

    def _B_ref(x, k_cache, v_cache, wq, wo):
        B, Sq, D = x.shape
        Hq, Dh = 32, 128
        Hkv = k_cache.shape[1]
        rep = Hq // Hkv
        q = (lambda x, *d: x.transpose(*d))((x @ wq).reshape(B, Sq, Hq, Dh), 0, 2, 1, 3)
        k = jnp.repeat(k_cache, rep, axis=1)
        v = jnp.repeat(v_cache, rep, axis=1)
        scores = jnp.einsum("bhqd,bhkd->bhqk", q, k) * (Dh ** -0.5)
        p = _softmax(scores, axis=-1)
        o = jnp.einsum("bhqk,bhkd->bhqd", p, v)
        return (lambda x, *d: x.transpose(*d))(o, 0, 2, 1, 3).reshape(B, Sq, Hq * Dh) @ wo

    a = _A_ref(A_x, A_k_cache, A_v_cache, A_wq, A_wo)
    b = _B_ref(B_x, B_k_cache, B_v_cache, B_wq, B_wo)
    return jnp.concatenate([a, b], axis=-1)
```

```python
import functools
import jax
import jax.numpy as jnp
from jax import lax
import jax.experimental.pallas as pl
import jax.experimental.pallas.tpu as pltpu

B, SQ, D = 8, 128, 576
HQ, HKV, SK, DH = 32, 16, 512, 128
REP = HQ // HKV
GW = REP * DH
M = B * SQ
NSTEP = 2 * HKV
DA = 512
NKV, NWQ, NWO = 4, 4, 5
NT = (((1,), (1,)), ((), ()))
F32 = jnp.float32
BF16 = jnp.bfloat16


def _kernel(ax, ak, av, awq, awo, bx, bk, bv, bwq, bwo, out_hbm,
            xt_buf, k_buf, v_buf, wq_buf, wo_buf, x_scr, q_scr, o_scr, acc_ref, out_buf,
            kv_sems, wq_sems, wo_sems, xsems, osems):
    scale = DH ** -0.5

    def kv_copies(k_hbm, v_hbm, h, slot):
        return (
            pltpu.make_async_copy(k_hbm.at[:, h], k_buf.at[slot], kv_sems.at[slot, 0]),
            pltpu.make_async_copy(v_hbm.at[:, h], v_buf.at[slot], kv_sems.at[slot, 1]),
        )

    def w_copy(w_hbm, buf, sems, h, slot):
        col = h * GW if isinstance(h, int) else pl.multiple_of(h * GW, GW)
        return pltpu.make_async_copy(w_hbm.at[:, pl.ds(col, GW)], buf.at[slot], sems.at[slot])

    def x_copy(x_hbm, i):
        return pltpu.make_async_copy(x_hbm, xt_buf.at[i], xsems.at[i])

    def outa_copy():
        return pltpu.make_async_copy(out_buf.at[:, 0:DA], out_hbm.at[:, 0:DA], osems.at[B])

    def outb_copy(b):
        rows = slice(b * SQ, (b + 1) * SQ)
        return pltpu.make_async_copy(out_buf.at[rows, DA:2 * D], out_hbm.at[rows, DA:2 * D], osems.at[b])

    def on_branch(t, fn_a, fn_b):
        if isinstance(t, int):
            if t < HKV:
                fn_a(t)
            elif t < NSTEP:
                fn_b(t - HKV)
        else:
            pl.when(t < HKV)(lambda: fn_a(t))
            pl.when(jnp.logical_and(t >= HKV, t < NSTEP))(lambda: fn_b(t - HKV))

    def rem(t, n):
        return t % n if isinstance(t, int) else lax.rem(t, n)

    def start_kv(t):
        sl = rem(t, NKV)

        def go(k_hbm, v_hbm):
            def f(h):
                for c in kv_copies(k_hbm, v_hbm, h, sl):
                    c.start()
            return f
        on_branch(t, go(ak, av), go(bk, bv))

    def start_wq(t):
        sl = rem(t, NWQ)
        on_branch(t, lambda h: w_copy(awq, wq_buf, wq_sems, h, sl).start(),
                  lambda h: w_copy(bwq, wq_buf, wq_sems, h, sl).start())

    def start_wo(t):
        sl = rem(t, NWO)
        on_branch(t, lambda h: w_copy(awo, wo_buf, wo_sems, h, sl).start(),
                  lambda h: w_copy(bwo, wo_buf, wo_sems, h, sl).start())

    def wait_kv(t):
        for c in kv_copies(ak, av, 0, rem(t, NKV)):
            c.wait()

    def wait_wq(t):
        w_copy(awq, wq_buf, wq_sems, 0, rem(t, NWQ)).wait()

    def wait_wo(t):
        w_copy(awo, wo_buf, wo_sems, 0, rem(t, NWO)).wait()

    def branch_of(t):
        return int(t >= HKV) if isinstance(t, int) else (t >= HKV).astype(jnp.int32)

    def transpose_x(i, b):
        x_scr[i, b * SQ:(b + 1) * SQ, :] = xt_buf[i, b].astype(F32).T.astype(BF16)

    def qproj(t, b):
        rows = slice(b * SQ, (b + 1) * SQ)
        q = jnp.dot(x_scr[branch_of(t), rows, :], wq_buf[rem(t, NWQ)], preferred_element_type=F32)
        q_scr[rows, :] = (q * scale).astype(BF16)

    def oproj(t, b):
        cols = slice(b * SQ, (b + 1) * SQ)
        acc_ref[branch_of(t), :, cols] += lax.dot_general(
            wo_buf[rem(t, NWO)], o_scr[cols, :], NT, preferred_element_type=F32)

    def qk(t, b):
        qb = jnp.concatenate(
            [q_scr[b * SQ:(b + 1) * SQ, g * DH:(g + 1) * DH] for g in range(REP)], axis=0)
        return lax.dot_general(qb, k_buf[rem(t, NKV), b], NT, preferred_element_type=F32)

    def softmax_pv(t, b, s_):
        m = jnp.max(s_, axis=-1, keepdims=True)
        p = jnp.exp(s_ - m)
        l = jnp.sum(p, axis=-1, keepdims=True)
        o = jnp.dot(p.astype(BF16), v_buf[rem(t, NKV), b], preferred_element_type=F32)
        r = pl.reciprocal(l, approx=True)
        r = r * (2.0 - l * r)
        o = (o * r).astype(BF16)
        for g in range(REP):
            o_scr[b * SQ:(b + 1) * SQ, g * DH:(g + 1) * DH] = o[g * SQ:(g + 1) * SQ]

    def finalize(br, b):
        rows = slice(b * SQ, (b + 1) * SQ)
        out_buf[rows, br * D:(br + 1) * D] = acc_ref[br, :, rows].T.astype(BF16)

    x_copy(ax, 0).start()
    start_wq(0)
    start_kv(0)
    start_wq(1)
    start_wo(0)
    acc_ref[...] = jnp.zeros((2, D, M), F32)
    x_copy(ax, 0).wait()
    for b in range(B):
        transpose_x(0, b)
    wait_wq(0)
    for b in range(B):
        qproj(0, b)

    wait_kv(0)
    wait_wo(0)
    wait_wq(1)
    for b in range(B):
        s_ = qk(0, b)
        if b == 0:
            start_kv(1)
            start_kv(2)
            start_wq(2)
            start_wo(1)
            start_wq(3)
            start_wo(2)
        qproj(1, b)
        if b >= 1:
            oproj(0, b - 1)
        softmax_pv(0, b, s_)

    def body(i, carry):
        s = 2 * i + 1

        @pl.when(i == 1)
        def _():
            x_copy(bx, 1).start()

        @pl.when(i == 4)
        def _():
            x_copy(bx, 1).wait()
            for b in range(B):
                transpose_x(1, b)

        wait_kv(s)
        wait_kv(s + 1)
        wait_wo(s)
        wait_wo(s + 1)
        wait_wq(s + 1)
        wait_wq(s + 2)
        for j in range(2):
            t = s + j
            for b in range(B):
                s_ = qk(t, b)
                if j == 0 and b == 0:
                    start_kv(s + 2)
                    start_kv(s + 3)
                    start_wo(s + 2)
                    start_wo(s + 3)
                    start_wq(s + 3)
                    start_wq(s + 4)
                qproj(t + 1, b)
                if b >= 1:
                    oproj(t, b - 1)
                else:
                    oproj(t - 1, B - 1)
                softmax_pv(t, b, s_)
        return carry

    lax.fori_loop(0, (NSTEP - 2) // 2, body, 0)

    s = NSTEP - 1
    wait_kv(s)
    wait_wo(s)
    s_cur = qk(s, 0)
    for b in range(B):
        s_nxt = qk(s, b + 1) if b + 1 < B else None
        if b >= 1:
            oproj(s, b - 1)
        else:
            oproj(s - 1, B - 1)
        if b < B // 2:
            finalize(0, 2 * b)
            finalize(0, 2 * b + 1)
            if b == B // 2 - 1:
                outa_copy().start()
        if b >= 2:
            finalize(1, b - 2)
            outb_copy(b - 2).start()
        softmax_pv(s, b, s_cur)
        s_cur = s_nxt
    finalize(1, B - 2)
    outb_copy(B - 2).start()
    oproj(s, B - 1)
    finalize(1, B - 1)
    outb_copy(B - 1).start()
    outa_copy().wait()
    for b in range(B):
        outb_copy(b).wait()


@jax.jit
def pallas_concat_heads__gqa_block_cached__gqa_block_cached__near_ridge_kernel(
    A_x, A_k_cache, A_v_cache, A_wq, A_wo, B_x, B_k_cache, B_v_cache, B_wq, B_wo):
    ax = jnp.swapaxes(A_x, 1, 2)
    bx = jnp.swapaxes(B_x, 1, 2)
    awo = A_wo.T
    bwo = B_wo.T
    out = pl.pallas_call(
        _kernel,
        in_specs=[pl.BlockSpec(memory_space=pl.ANY)] * 10,
        out_specs=pl.BlockSpec(memory_space=pl.ANY),
        out_shape=jax.ShapeDtypeStruct((M, 2 * D), BF16),
        scratch_shapes=[
            pltpu.VMEM((2, B, D, SQ), BF16),
            pltpu.VMEM((NKV, B, SK, DH), BF16),
            pltpu.VMEM((NKV, B, SK, DH), BF16),
            pltpu.VMEM((NWQ, D, GW), BF16),
            pltpu.VMEM((NWO, D, GW), BF16),
            pltpu.VMEM((2, M, D), BF16),
            pltpu.VMEM((M, GW), BF16),
            pltpu.VMEM((M, GW), BF16),
            pltpu.VMEM((2, D, M), F32),
            pltpu.VMEM((M, 2 * D), BF16),
            pltpu.SemaphoreType.DMA((NKV, 2)),
            pltpu.SemaphoreType.DMA((NWQ,)),
            pltpu.SemaphoreType.DMA((NWO,)),
            pltpu.SemaphoreType.DMA((2,)),
            pltpu.SemaphoreType.DMA((B + 1,)),
        ],
        compiler_params=pltpu.CompilerParams(
            vmem_limit_bytes=96 * 1024 * 1024,
            disable_bounds_checks=True,
        ),
    )(ax, A_k_cache, A_v_cache, A_wq, awo, bx, B_k_cache, B_v_cache, B_wq, bwo)
    return out.reshape(B, SQ, 2 * D)
```

```python
import jax
import jax.numpy as jnp
from jax import lax
import jax.experimental.pallas as pl
import jax.experimental.pallas.tpu as pltpu

B, SQ, D = 8, 128, 576
HQ, HKV, SK, DH = 32, 16, 512, 128
REP = HQ // HKV
GW = REP * DH
M = B * SQ
NSTEP = 2 * HKV
DA = 512
NKV, NWQ, NWO = 4, 4, 8
NT = (((1,), (1,)), ((), ()))
F32 = jnp.float32
BF16 = jnp.bfloat16


def _kernel(ax, ak, av, awq, awo, bx, bk, bv, bwq, bwo, out_hbm,
            xt_buf, k_buf, v_buf, wq_buf, wo_buf, x_scr, q_scr, o_scr, acc_ref, out_buf,
            kv_sems, wq_sems, wo_sems, xsems, osems):
    scale = DH ** -0.5

    def kv_copies(k_hbm, v_hbm, h, slot):
        return (
            pltpu.make_async_copy(k_hbm.at[:, h], k_buf.at[slot], kv_sems.at[slot, 0]),
            pltpu.make_async_copy(v_hbm.at[:, h], v_buf.at[slot], kv_sems.at[slot, 1]),
        )

    def w_copy(w_hbm, buf, sems, h, slot):
        col = h * GW if isinstance(h, int) else pl.multiple_of(h * GW, GW)
        return pltpu.make_async_copy(w_hbm.at[:, pl.ds(col, GW)], buf.at[slot], sems.at[slot])

    def x_copy(x_hbm, i):
        return pltpu.make_async_copy(x_hbm, xt_buf.at[i], xsems.at[i])

    def outa_copy():
        return pltpu.make_async_copy(out_buf.at[:, 0:DA], out_hbm.at[:, 0:DA], osems.at[B])

    def outb_copy(b):
        rows = slice(b * SQ, (b + 1) * SQ)
        return pltpu.make_async_copy(out_buf.at[rows, DA:2 * D], out_hbm.at[rows, DA:2 * D],
                                     osems.at[b])

    def on_branch(t, fn_a, fn_b):
        if isinstance(t, int):
            if t < HKV:
                fn_a(t)
            elif t < NSTEP:
                fn_b(t - HKV)
        else:
            pl.when(t < HKV)(lambda: fn_a(t))
            pl.when(jnp.logical_and(t >= HKV, t < NSTEP))(lambda: fn_b(t - HKV))

    def rem(t, n):
        return t % n if isinstance(t, int) else jnp.bitwise_and(t, n - 1)

    def branch_of(t):
        return int(t >= HKV) if isinstance(t, int) else (t >= HKV).astype(jnp.int32)

    def start_kv(t):
        sl = rem(t, NKV)

        def go(k_hbm, v_hbm):
            def f(h):
                for c in kv_copies(k_hbm, v_hbm, h, sl):
                    c.start()
            return f
        on_branch(t, go(ak, av), go(bk, bv))

    def start_wq(t):
        sl = rem(t, NWQ)
        on_branch(t, lambda h: w_copy(awq, wq_buf, wq_sems, h, sl).start(),
                  lambda h: w_copy(bwq, wq_buf, wq_sems, h, sl).start())

    def start_wo(t):
        sl = rem(t, NWO)
        on_branch(t, lambda h: w_copy(awo, wo_buf, wo_sems, h, sl).start(),
                  lambda h: w_copy(bwo, wo_buf, wo_sems, h, sl).start())

    def wait_kv(t):
        for c in kv_copies(ak, av, 0, rem(t, NKV)):
            c.wait()

    def wait_wq(t):
        w_copy(awq, wq_buf, wq_sems, 0, rem(t, NWQ)).wait()

    def wait_wo(t):
        w_copy(awo, wo_buf, wo_sems, 0, rem(t, NWO)).wait()

    def start_group(t):
        def f():
            start_kv(t)
            start_wq(t + 1)
            start_wo(t)
        return f

    def transpose_x(i, b):
        x_scr[i, b * SQ:(b + 1) * SQ, :] = xt_buf[i, b].astype(F32).T.astype(BF16)

    def qproj(t, b):
        rows = slice(b * SQ, (b + 1) * SQ)
        q = jnp.dot(x_scr[branch_of(t), rows, :], wq_buf[rem(t, NWQ)], preferred_element_type=F32)
        q_scr[rows, :] = (q * scale).astype(BF16)

    def oproj(t, b):
        cols = slice(b * SQ, (b + 1) * SQ)
        acc_ref[branch_of(t), :, cols] += lax.dot_general(
            wo_buf[rem(t, NWO)], o_scr[cols, :], NT, preferred_element_type=F32)

    def qk(t, b):
        qb = jnp.concatenate(
            [q_scr[b * SQ:(b + 1) * SQ, g * DH:(g + 1) * DH] for g in range(REP)], axis=0)
        return lax.dot_general(qb, k_buf[rem(t, NKV), b], NT, preferred_element_type=F32)

    def softmax_pv(t, b, s_):
        m = jnp.max(s_, axis=-1, keepdims=True)
        p = jnp.exp(s_ - m)
        l = jnp.sum(p, axis=-1, keepdims=True)
        o = jnp.dot(p.astype(BF16), v_buf[rem(t, NKV), b], preferred_element_type=F32)
        r = pl.reciprocal(l, approx=True)
        r = r * (2.0 - l * r)
        o = (o * r).astype(BF16)
        for g in range(REP):
            o_scr[b * SQ:(b + 1) * SQ, g * DH:(g + 1) * DH] = o[g * SQ:(g + 1) * SQ]

    def finalize(br, b):
        rows = slice(b * SQ, (b + 1) * SQ)
        out_buf[rows, br * D:(br + 1) * D] = acc_ref[br, :, rows].T.astype(BF16)

    def regular_units(t, first=False, hooks=None):
        for b in range(B):
            s_ = qk(t, b)
            if hooks is not None and b in hooks:
                hooks[b]()
            qproj(t + 1, b)
            if b >= 1:
                oproj(t, b - 1)
            elif not first:
                oproj(t - 1, B - 1)
            softmax_pv(t, b, s_)

    x_copy(ax, 0).start()
    start_wq(0)
    start_kv(0)
    start_wq(1)
    start_wo(0)
    acc_ref[...] = jnp.zeros((2, D, M), F32)
    x_copy(ax, 0).wait()
    for b in range(B):
        transpose_x(0, b)
    wait_wq(0)
    for b in range(B):
        qproj(0, b)

    wait_kv(0)
    wait_wo(0)
    wait_wq(1)
    regular_units(0, first=True, hooks={0: start_group(1), 5: start_group(2)})
    wait_kv(1)
    wait_wo(1)
    wait_wq(2)
    regular_units(1, hooks={2: start_group(3)})

    def body(i, carry):
        s = 2 * i + 2

        @pl.when(i == 1)
        def _():
            x_copy(bx, 1).start()

        @pl.when(i == 4)
        def _():
            x_copy(bx, 1).wait()
            for b in range(B):
                transpose_x(1, b)

        wait_kv(s)
        wait_kv(s + 1)
        wait_wo(s)
        wait_wo(s + 1)
        wait_wq(s + 1)
        wait_wq(s + 2)

        def prefetch():
            start_kv(s + 2)
            start_kv(s + 3)
            start_wo(s + 2)
            start_wo(s + 3)
            start_wq(s + 3)
            start_wq(s + 4)
        regular_units(s, hooks={0: prefetch})
        regular_units(s + 1)
        return carry

    lax.fori_loop(0, (NSTEP - 4) // 2, body, 0)

    s = NSTEP - 1
    wait_kv(s - 1)
    wait_kv(s)
    wait_wo(s - 1)
    wait_wo(s)
    wait_wq(s)
    regular_units(s - 1)
    s_cur = qk(s, 0)
    for b in range(B):
        s_nxt = qk(s, b + 1) if b + 1 < B else None
        if b >= 1:
            oproj(s, b - 1)
        else:
            oproj(s - 1, B - 1)
        if b < B // 2:
            finalize(0, 2 * b)
            finalize(0, 2 * b + 1)
            if b == B // 2 - 1:
                outa_copy().start()
        if b >= 2:
            finalize(1, b - 2)
            outb_copy(b - 2).start()
        softmax_pv(s, b, s_cur)
        s_cur = s_nxt
    finalize(1, B - 2)
    outb_copy(B - 2).start()
    oproj(s, B - 1)
    finalize(1, B - 1)
    outb_copy(B - 1).start()
    outa_copy().wait()
    for b in range(B):
        outb_copy(b).wait()


@jax.jit
def pallas_concat_heads__gqa_block_cached__gqa_block_cached__near_ridge_kernel(
    A_x: jax.Array,
    A_k_cache: jax.Array,
    A_v_cache: jax.Array,
    A_wq: jax.Array,
    A_wo: jax.Array,
    B_x: jax.Array,
    B_k_cache: jax.Array,
    B_v_cache: jax.Array,
    B_wq: jax.Array,
    B_wo: jax.Array,
):
    ax = jnp.swapaxes(A_x, 1, 2)
    bx = jnp.swapaxes(B_x, 1, 2)
    awo = A_wo.T
    bwo = B_wo.T
    out = pl.pallas_call(
        _kernel,
        in_specs=[pl.BlockSpec(memory_space=pl.ANY)] * 10,
        out_specs=pl.BlockSpec(memory_space=pl.ANY),
        out_shape=jax.ShapeDtypeStruct((M, 2 * D), BF16),
        scratch_shapes=[
            pltpu.VMEM((2, B, D, SQ), BF16),
            pltpu.VMEM((NKV, B, SK, DH), BF16),
            pltpu.VMEM((NKV, B, SK, DH), BF16),
            pltpu.VMEM((NWQ, D, GW), BF16),
            pltpu.VMEM((NWO, D, GW), BF16),
            pltpu.VMEM((2, M, D), BF16),
            pltpu.VMEM((M, GW), BF16),
            pltpu.VMEM((M, GW), BF16),
            pltpu.VMEM((2, D, M), F32),
            pltpu.VMEM((M, 2 * D), BF16),
            pltpu.SemaphoreType.DMA((NKV, 2)),
            pltpu.SemaphoreType.DMA((NWQ,)),
            pltpu.SemaphoreType.DMA((NWO,)),
            pltpu.SemaphoreType.DMA((2,)),
            pltpu.SemaphoreType.DMA((B + 1,)),
        ],
        compiler_params=pltpu.CompilerParams(
            vmem_limit_bytes=96 * 1024 * 1024,
            disable_bounds_checks=True,
        ),
    )(ax, A_k_cache, A_v_cache, A_wq, awo, bx, B_k_cache, B_v_cache, B_wq, bwo)
    return out.reshape(B, SQ, 2 * D)
```
